```python
import os as _os
_os.environ.setdefault("JAX_PLATFORMS", "cpu")
import jax
import jax.numpy as jnp

def _softmax(x, axis=-1):
    return jax.nn.softmax(x, axis=axis)
def _gelu(x):
    return jax.nn.gelu(x, approximate=True)
def _silu(x):
    return jax.nn.silu(x)
def _sigmoid(x):
    return jax.nn.sigmoid(x)
def _layernorm(x, axis=-1, eps=1e-5):
    m = jnp.mean(x, axis=axis, keepdims=True)
    v = jnp.var(x, axis=axis, keepdims=True)
    return (x - m) / jnp.sqrt(v + eps)
def _scatter_add(tgt, idx, src, axis=0):
    return tgt.at[idx].add(src)
def _segment_sum(src, seg, n):
    return jax.ops.segment_sum(src, seg, n)
class _Rng:
    def __init__(self, key):
        self._k = key
    def _next(self):
        self._k, sub = jax.random.split(self._k)
        return sub
    def normal(self, shape):
        return jax.random.normal(self._next(), shape, dtype=jnp.bfloat16)
    def randint(self, lo, hi, shape):
        return jax.random.randint(self._next(), shape, lo, hi, dtype=jnp.int32)
    def uniform(self, shape, lo=0.0, hi=1.0):
        return jax.random.uniform(self._next(), shape, jnp.bfloat16, lo, hi)
    def permutation(self, n):
        return jax.random.permutation(self._next(), n)


kernel_name = 'standalone__mha_softmax__near_ridge'

def setup_inputs():
    _rng = _Rng(jax.random.key(int.from_bytes(__import__("os").urandom(4), "little")))
    _w = (lambda a: (lambda t: t.astype(jnp.bfloat16) if jnp.issubdtype(t.dtype, jnp.floating) else t)(jnp.asarray(a)))
    B, H, Sq, Sk, D = 8, 32, 304, 2048, 128
    return {
        "q": _w((lambda *s: _rng.normal(s) * 0.4)(B, H, Sq, D)),
        "k": _w((lambda *s: _rng.normal(s) * 0.4)(B, H, Sk, D)),
        "v": _w((lambda *s: _rng.normal(s) * 0.05)(B, H, Sk, D)),
    }

def reference(q, k, v):
    scale = q.shape[-1] ** -0.5
    scores = jnp.einsum("bhqd,bhkd->bhqk", q, k) * scale
    p = _softmax(scores, axis=-1)
    return jnp.einsum("bhqk,bhkd->bhqd", p, v)
```

```python
import functools
import jax
import jax.numpy as jnp
from jax import lax
import jax.experimental.pallas as pl
import jax.experimental.pallas.tpu as pltpu


def _attn_kernel(q_ref, k_ref, v_ref, o_ref, *, scale, hb):
    for h in range(hb):
        q = q_ref[0, h]
        k = k_ref[0, h]
        s = lax.dot_general(q, k, (((1,), (1,)), ((), ())),
                            preferred_element_type=jnp.float32)
        s = s * scale
        m = jnp.max(s, axis=-1, keepdims=True)
        p = jnp.exp(s - m)
        l = jnp.sum(p, axis=-1, keepdims=True)
        o = jnp.dot(p.astype(jnp.bfloat16), v_ref[0, h],
                    preferred_element_type=jnp.float32)
        o_ref[0, h] = (o / l).astype(o_ref.dtype)


@functools.partial(jax.jit, static_argnames=("hb",))
def pallas_standalone__mha_softmax__near_ridge_kernel(q, k, v, hb=1):
    B, H, Sq, D = q.shape
    Sk = k.shape[2]
    scale = D ** -0.5
    kernel = functools.partial(_attn_kernel, scale=scale, hb=hb)
    return pl.pallas_call(
        kernel,
        grid=(B, H // hb),
        in_specs=[
            pl.BlockSpec((1, hb, Sq, D), lambda b, h: (b, h, 0, 0)),
            pl.BlockSpec((1, hb, Sk, D), lambda b, h: (b, h, 0, 0)),
            pl.BlockSpec((1, hb, Sk, D), lambda b, h: (b, h, 0, 0)),
        ],
        out_specs=pl.BlockSpec((1, hb, Sq, D), lambda b, h: (b, h, 0, 0)),
        out_shape=jax.ShapeDtypeStruct((B, H, Sq, D), q.dtype),
        compiler_params=pltpu.CompilerParams(
            dimension_semantics=("parallel", "parallel"),
            vmem_limit_bytes=100 * 1024 * 1024,
        ),
    )(q, k, v)
```

```python
import functools
import jax
import jax.numpy as jnp
from jax import lax
import jax.experimental.pallas as pl
import jax.experimental.pallas.tpu as pltpu

LOG2E = 1.4426950408889634


def _one_head(q_ref, k_ref, v_ref, o_ref, scale, gk):
    Sq, D = q_ref.shape
    Sk = k_ref.shape[0]
    ng = Sk // gk
    nt = gk // 128
    c = scale * LOG2E
    q = q_ref[...]
    mc_old = None
    acc = None
    l_run = None
    for g in range(ng):
        kg = k_ref[pl.ds(g * gk, gk), :]
        s = lax.dot_general(q, kg, (((1,), (1,)), ((), ())),
                            preferred_element_type=jnp.float32)
        mg = s[:, 0:128]
        for t in range(1, nt):
            mg = jnp.maximum(mg, s[:, t * 128:(t + 1) * 128])
        mc_g = jnp.max(mg, axis=-1, keepdims=True) * c
        if mc_old is None:
            mc_new = mc_g
        else:
            mc_new = jnp.maximum(mc_old, mc_g)
        p = jnp.exp2(s * c - mc_new)
        lg = p[:, 0:128]
        for t in range(1, nt):
            lg = lg + p[:, t * 128:(t + 1) * 128]
        pv = jnp.dot(p.astype(jnp.bfloat16), v_ref[pl.ds(g * gk, gk), :],
                     preferred_element_type=jnp.float32)
        if mc_old is None:
            acc = pv
            l_run = lg
        else:
            alpha = jnp.exp2(mc_old - mc_new)
            acc = acc * alpha + pv
            l_run = l_run * alpha + lg
        mc_old = mc_new
    l = jnp.sum(l_run, axis=-1, keepdims=True)
    r0 = pl.reciprocal(l, approx=True)
    inv_l = r0 * (2.0 - l * r0)
    o_ref[...] = (acc * inv_l).astype(o_ref.dtype)


def _attn_kernel(q_ref, k_ref, v_ref, o_ref, *, scale, gk, hb):
    for h in range(hb):
        _one_head(q_ref.at[h], k_ref.at[h], v_ref.at[h], o_ref.at[h], scale, gk)


@functools.partial(jax.jit, static_argnames=("gk", "hb"))
def pallas_standalone__mha_softmax__near_ridge_kernel(q, k, v, gk=512, hb=4):
    B, H, Sq, D = q.shape
    Sk = k.shape[2]
    scale = D ** -0.5
    kernel = functools.partial(_attn_kernel, scale=scale, gk=gk, hb=hb)
    return pl.pallas_call(
        kernel,
        grid=(B, H // hb),
        in_specs=[
            pl.BlockSpec((None, hb, Sq, D), lambda b, h: (b, h, 0, 0)),
            pl.BlockSpec((None, hb, Sk, D), lambda b, h: (b, h, 0, 0)),
            pl.BlockSpec((None, hb, Sk, D), lambda b, h: (b, h, 0, 0)),
        ],
        out_specs=pl.BlockSpec((None, hb, Sq, D), lambda b, h: (b, h, 0, 0)),
        out_shape=jax.ShapeDtypeStruct((B, H, Sq, D), q.dtype),
        compiler_params=pltpu.CompilerParams(
            dimension_semantics=("parallel", "parallel"),
            vmem_limit_bytes=100 * 1024 * 1024,
        ),
    )(q, k, v)
```

```python
import functools

import jax
import jax.numpy as jnp
from jax import lax
import jax.experimental.pallas as pl
import jax.experimental.pallas.tpu as pltpu

LOG2E = 1.4426950408889634


def _attention_one_head(q_ref, k_ref, v_ref, o_ref, scale, gk):
    Sk = k_ref.shape[0]
    ng = Sk // gk
    nt = gk // 128
    c = scale * LOG2E
    q = (q_ref[...].astype(jnp.float32) * c).astype(q_ref.dtype)
    m_old = None
    acc = None
    l_run = None
    for g in range(ng):
        kg = k_ref[pl.ds(g * gk, gk), :]
        s = lax.dot_general(q, kg, (((1,), (1,)), ((), ())),
                            preferred_element_type=jnp.float32)
        mg = s[:, 0:128]
        for t in range(1, nt):
            mg = jnp.maximum(mg, s[:, t * 128:(t + 1) * 128])
        m_g = jnp.max(mg, axis=-1, keepdims=True)
        m_new = m_g if m_old is None else jnp.maximum(m_old, m_g)
        p = jnp.exp2(s - m_new)
        lg = p[:, 0:128]
        for t in range(1, nt):
            lg = lg + p[:, t * 128:(t + 1) * 128]
        pv = jnp.dot(p.astype(jnp.bfloat16), v_ref[pl.ds(g * gk, gk), :],
                     preferred_element_type=jnp.float32)
        if m_old is None:
            acc, l_run = pv, lg
        else:
            alpha = jnp.exp2(m_old - m_new)
            acc = acc * alpha + pv
            l_run = l_run * alpha + lg
        m_old = m_new
    l = jnp.sum(l_run, axis=-1, keepdims=True)
    r0 = pl.reciprocal(l, approx=True)
    inv_l = r0 * (2.0 - l * r0)
    o_ref[...] = (acc * inv_l).astype(o_ref.dtype)


def _attention_kernel(q_hbm, k_hbm, v_hbm, o_hbm, qbuf, kbuf, vbuf, obuf,
                      qsem, ksem, vsem, osem, *, scale, gk, hb, ns):
    nblk = q_hbm.shape[0] // hb

    def in_copies(blk, slot):
        return (pltpu.make_async_copy(q_hbm.at[pl.ds(blk * hb, hb)], qbuf.at[slot], qsem.at[slot]),
                pltpu.make_async_copy(k_hbm.at[pl.ds(blk * hb, hb)], kbuf.at[slot], ksem.at[slot]),
                pltpu.make_async_copy(v_hbm.at[pl.ds(blk * hb, hb)], vbuf.at[slot], vsem.at[slot]))

    def out_copy(blk, slot):
        return pltpu.make_async_copy(obuf.at[slot], o_hbm.at[pl.ds(blk * hb, hb)], osem.at[slot])

    for s in range(ns - 1):
        for cp in in_copies(s, s):
            cp.start()

    def body(b, carry):
        slot = b & (ns - 1)
        oslot = b & 1

        for cp in in_copies(b, slot):
            cp.wait()

        @pl.when(b >= 2)
        def _():
            out_copy(b - 2, oslot).wait()

        for h in range(hb):
            _attention_one_head(qbuf.at[slot, h], kbuf.at[slot, h], vbuf.at[slot, h],
                                obuf.at[oslot, h], scale, gk)
            if h == 0:
                nxt = b + (ns - 1)

                @pl.when(nxt < nblk)
                def _():
                    for cp in in_copies(nxt, nxt & (ns - 1)):
                        cp.start()

        out_copy(b, oslot).start()
        return carry

    lax.fori_loop(0, nblk, body, 0)

    for b in (nblk - 2, nblk - 1):
        out_copy(b, b & 1).wait()


@jax.jit
def pallas_standalone__mha_softmax__near_ridge_kernel(
    q: jax.Array,
    k: jax.Array,
    v: jax.Array,
):
    B, H, Sq, D = q.shape
    Sk = k.shape[2]
    N = B * H
    gk, hb, ns = 512, 4, 4
    assert N % hb == 0 and N // hb >= 2 and Sk % gk == 0 and gk % 128 == 0
    scale = D ** -0.5
    kernel = functools.partial(_attention_kernel, scale=scale, gk=gk, hb=hb, ns=ns)
    out = pl.pallas_call(
        kernel,
        in_specs=[
            pl.BlockSpec(memory_space=pl.ANY),
            pl.BlockSpec(memory_space=pl.ANY),
            pl.BlockSpec(memory_space=pl.ANY),
        ],
        out_specs=pl.BlockSpec(memory_space=pl.ANY),
        out_shape=jax.ShapeDtypeStruct((N, Sq, D), q.dtype),
        scratch_shapes=[
            pltpu.VMEM((ns, hb, Sq, D), q.dtype),
            pltpu.VMEM((ns, hb, Sk, D), k.dtype),
            pltpu.VMEM((ns, hb, Sk, D), v.dtype),
            pltpu.VMEM((2, hb, Sq, D), q.dtype),
            pltpu.SemaphoreType.DMA((ns,)),
            pltpu.SemaphoreType.DMA((ns,)),
            pltpu.SemaphoreType.DMA((ns,)),
            pltpu.SemaphoreType.DMA((2,)),
        ],
        compiler_params=pltpu.CompilerParams(
            vmem_limit_bytes=100 * 1024 * 1024,
        ),
    )(q.reshape(N, Sq, D), k.reshape(N, Sk, D), v.reshape(N, Sk, D))
    return out.reshape(B, H, Sq, D)
```
